```python
import os as _os
_os.environ.setdefault("JAX_PLATFORMS", "cpu")
import jax
import jax.numpy as jnp

def _softmax(x, axis=-1):
    return jax.nn.softmax(x, axis=axis)
def _gelu(x):
    return jax.nn.gelu(x, approximate=True)
def _silu(x):
    return jax.nn.silu(x)
def _sigmoid(x):
    return jax.nn.sigmoid(x)
def _layernorm(x, axis=-1, eps=1e-5):
    m = jnp.mean(x, axis=axis, keepdims=True)
    v = jnp.var(x, axis=axis, keepdims=True)
    return (x - m) / jnp.sqrt(v + eps)
def _scatter_add(tgt, idx, src, axis=0):
    return tgt.at[idx].add(src)
def _segment_sum(src, seg, n):
    return jax.ops.segment_sum(src, seg, n)
class _Rng:
    def __init__(self, key):
        self._k = key
    def _next(self):
        self._k, sub = jax.random.split(self._k)
        return sub
    def normal(self, shape):
        return jax.random.normal(self._next(), shape, dtype=jnp.bfloat16)
    def randint(self, lo, hi, shape):
        return jax.random.randint(self._next(), shape, lo, hi, dtype=jnp.int32)
    def uniform(self, shape, lo=0.0, hi=1.0):
        return jax.random.uniform(self._next(), shape, jnp.bfloat16, lo, hi)
    def permutation(self, n):
        return jax.random.permutation(self._next(), n)


kernel_name = 'gated_mix__ssm_conv_s5__geglu_ffn__prompt'

def setup_inputs():
    _rng = _Rng(jax.random.key(int.from_bytes(__import__("os").urandom(4), "little")))
    _w = (lambda a: (lambda t: t.astype(jnp.bfloat16) if jnp.issubdtype(t.dtype, jnp.floating) else t)(jnp.asarray(a)))
    def _A_setup():
        B, S, D = 1, 2048, 512
        P = D
        Lambda_re = -0.5 * jnp.exp((lambda *s: _rng.normal(s) * 0.4)(P))
        Lambda_im = (lambda *s: _rng.normal(s) * 0.4)(P) * 1.0
        B_re = (lambda *s: _rng.normal(s) * 0.4)(P, D) * (D ** -0.5)
        B_im = (lambda *s: _rng.normal(s) * 0.4)(P, D) * (D ** -0.5)
        C_re = (lambda *s: _rng.normal(s) * 0.4)(D, P) * (P ** -0.5)
        C_im = (lambda *s: _rng.normal(s) * 0.4)(D, P) * (P ** -0.5)
        log_dt = (lambda *s: _rng.normal(s) * 0.4)(P) * 0.3 - 2.0
        Dskip = (lambda *s: _rng.normal(s) * 0.4)(D)
        return {
            "x": _w((lambda *s: _rng.normal(s) * 0.05)(B, S, D)),
            "Lambda_re": _w(Lambda_re),
            "Lambda_im": _w(Lambda_im),
            "B_re": _w(B_re),
            "B_im": _w(B_im),
            "C_re": _w(C_re),
            "C_im": _w(C_im),
            "log_dt": _w(log_dt),
            "Dskip": _w(Dskip),
        }
    _A_in = _A_setup()

    def _B_setup():
        B, S, D, F = 1, 2048, 512, 1376
        return {
            "x": _w((lambda *s: _rng.normal(s) * 0.05)(B, S, D)),
            "w_gate": _w((lambda *s: _rng.normal(s) * 0.1)(D, F)),
            "w_up": _w((lambda *s: _rng.normal(s) * 0.1)(D, F)),
            "w_down": _w((lambda *s: _rng.normal(s) * 0.1)(F, D)),
        }
    _B_in = _B_setup()

    return {
        "A_x": _A_in["x"],
        "A_Lambda_re": _A_in["Lambda_re"],
        "A_Lambda_im": _A_in["Lambda_im"],
        "A_B_re": _A_in["B_re"],
        "A_B_im": _A_in["B_im"],
        "A_C_re": _A_in["C_re"],
        "A_C_im": _A_in["C_im"],
        "A_log_dt": _A_in["log_dt"],
        "A_Dskip": _A_in["Dskip"],
        "B_x": _B_in["x"],
        "B_w_gate": _B_in["w_gate"],
        "B_w_up": _B_in["w_up"],
        "B_w_down": _B_in["w_down"],
        "gate_w": _w((lambda *s: _rng.normal(s) * 0.05)(512) * 16.0),
    }

def reference(A_x, A_Lambda_re, A_Lambda_im, A_B_re, A_B_im, A_C_re, A_C_im, A_log_dt, A_Dskip, B_x, B_w_gate, B_w_up, B_w_down, gate_w):
    def _A_ref(x, Lambda_re, Lambda_im, B_re, B_im, C_re, C_im, log_dt, Dskip):
        Bsz, L, H = x.shape
        Lam = Lambda_re + 1j * Lambda_im
        Bmat = B_re + 1j * B_im
        Cmat = C_re + 1j * C_im
        dt = jnp.exp(log_dt)
        Lam_bar = jnp.exp(dt * Lam)
        B_bar = ((Lam_bar - 1.0) / Lam)[:, None] * Bmat
        Bu = jnp.einsum("bld,pd->blp", x + 0j, B_bar)
        h = jnp.zeros_like(Bu[:, 0, :])
        hs = []
        for t in range(L):
            h = Lam_bar[None, :] * h + Bu[:, t, :]
            hs.append(h)
        hseq = jnp.stack(hs, 1)
        y = 2.0 * jnp.einsum("blp,dp->bld", hseq, Cmat).real + x * Dskip[None, None, :]
        return y

    def _B_ref(x, w_gate, w_up, w_down):
        return (_gelu(x @ w_gate) * (x @ w_up)) @ w_down

    x = A_x
    g = _sigmoid((x * gate_w).sum(-1, keepdims=True))
    a = _A_ref(x, A_Lambda_re, A_Lambda_im, A_B_re, A_B_im, A_C_re, A_C_im, A_log_dt, A_Dskip)
    b = _B_ref(x, B_w_gate, B_w_up, B_w_down)
    return g * a + (1 - g) * b
```

```python
import numpy as np
import jax
import jax.numpy as jnp
from jax import lax
import jax.experimental.pallas as pl
import jax.experimental.pallas.tpu as pltpu

f32 = jnp.float32
bf16 = jnp.bfloat16
DNT = (((1,), (1,)), ((), ()))

def _gelu(x):
    c = 0.7978845608028654
    return 0.5 * x * (1.0 + jnp.tanh(c * (x + 0.044715 * (x * x * x))))

def dnt(a, b):
    return lax.dot_general(a, b, DNT, preferred_element_type=f32)

def dnn(a, b):
    return jnp.dot(a, b, preferred_element_type=f32)

def s_comb(m):
    m1, m2, m3, m4, m5, m6, m7 = m
    return (m1 + m4) + (m7 - m5), m3 + m5, m2 + m4, (m1 - m2) + (m3 + m6)

def s_lhs32(a11, a12, a21, a22):
    return [a11 + a22, a21 + a22, a11, a22, a11 + a12, a21 - a11, a12 - a22]

def s_rhs32(b11, b12, b21, b22):
    return [b11 + b22, b11, b12 - b22, b21 - b11, b22, b11 + b12, b21 + b22]

def merge2(a, b):
    out = []; n = max(len(a), len(b))
    for k in range(n):
        out += a[k * len(a) // n:(k + 1) * len(a) // n] + b[k * len(b) // n:(k + 1) * len(b) // n]
    return out

def _build():
    TM, CW, dw = 256, 128, 2
    n6f, n7f = 0.5, 1.0
    zB = zG = zC = 6
    stagger = (3, 5, 7, 9)
    odt = jnp.float32
    S, D, P, F = 2048, 512, 512, 1376
    H = TM // 2
    KH = 256
    NB = S // TM
    L = TM // 8
    LP = L + 1
    SP = NB * 8 * LP
    T1 = 256
    NX = S // T1

    def kern(x_hbm, lre_hbm, lim_hbm, bre_hbm, bim_hbm, cre_hbm, cim_hbm, ldt_hbm, dsk_hbm,
             wg_hbm, wu_hbm, wd_hbm, gw_hbm, o_ref,
             x_s, lre_s, lim_s, ldt_s, dsk_s, gw_s, bre_s, bim_s, cre_s, cim_s, wg_s, wu_s, wd_s,
             bur_s, bui_s, xf_s, ot_s, tab_s, carry_s, vec_s, tf_s, tb_s, tc_s, hs_s, sb_s, b0r_s, b0i_s, sems):
        step = pl.program_id(0)

        def pos(i, rho):
            t = i * T1 + rho
            tt = t % TM
            return (t // TM) * (8 * LP) + (tt // L) * LP + (tt % L)

        def st4(ref, blk, rho, v):
            for a in range(0, v.shape[0], 8):
                off = pos(blk, rho + a)
                for k in range(4):
                    ref[k, pl.ds(off, 8), :] = v[a:a + 8, 128 * k:128 * k + 128]

        def ld(ref, pb, j):
            return jnp.concatenate([ref[k, pl.ds(pb + j, 8, stride=LP), :] for k in range(4)], 1)

        def zero_from(v):
            u = lax.bitcast_convert_type(v, jnp.uint32)
            u = lax.shift_right_logical(lax.shift_right_logical(u, np.uint32(31)), np.uint32(1))
            return lax.bitcast_convert_type(u, f32)

        def zero_bits(v, zdepth):
            u = lax.bitcast_convert_type(v, jnp.uint32)
            u = lax.shift_right_logical(u, np.uint32(31))
            for _ in range(zdepth - 1):
                u = lax.shift_right_logical(u, np.uint32(1))
            return u

        def gate16(v, zb):
            if zb is None:
                return v.astype(f32)
            return pltpu.bitcast(pltpu.bitcast(v, jnp.uint32) | zb, bf16).astype(f32)

        def scan_lane(blk, k, dep=None, bur_s=bur_s, bui_s=bui_s):
            pb = blk * (8 * LP)
            ks = slice(128 * k, 128 * k + 128)
            st = {}
            items = []
            ldk = lambda ref, j: ref[k, pl.ds(pb + j, 8, stride=LP), :]
            def first():
                st['lr'] = tab_s[0, :, ks]; st['li'] = tab_s[1, :, ks]
            def p1(j):
                def f():
                    br = ldk(bur_s, j); bi = ldk(bui_s, j)
                    if j == 0:
                        if dep is not None:
                            z = zero_from(dep())
                            br = br + z; bi = bi + z
                        st['h'] = (br, bi)
                    else:
                        hr, hi = st['h']; lr = st['lr']; li = st['li']
                        st['h'] = ((lr * hr - li * hi) + br, (lr * hi + li * hr) + bi)
                return f
            def carry():
                hr, hi = st['h']
                cr = carry_s[0, :, ks]; ci = carry_s[1, :, ks]
                row = lax.broadcasted_iota(jnp.int32, (8, 128), 0)
                LLr = tab_s[8, :, ks]; LLi = tab_s[9, :, ks]
                er = hr + (LLr * cr - LLi * ci); ei = hi + (LLr * ci + LLi * cr)
                for n, d in enumerate((1, 2, 4)):
                    sr = pltpu.roll(er, d, 0); si = pltpu.roll(ei, d, 0)
                    mr = tab_s[2 + 2 * n, :, ks]; mi = tab_s[3 + 2 * n, :, ks]
                    er, ei = er + (mr * sr - mi * si), ei + (mr * si + mi * sr)
                gr = jnp.where(row == 0, cr, pltpu.roll(er, 1, 0))
                gi = jnp.where(row == 0, ci, pltpu.roll(ei, 1, 0))
                carry_s[0, :, ks] = jnp.broadcast_to(er[7:8], (8, 128))
                carry_s[1, :, ks] = jnp.broadcast_to(ei[7:8], (8, 128))
                st['h'] = (gr, gi); st['o'] = []
            def p2(j):
                def f():
                    br = ldk(bur_s, j); bi = ldk(bui_s, j)
                    hr, hi = st['h']; lr = st['lr']; li = st['li']
                    hr, hi = (lr * hr - li * hi) + br, (lr * hi + li * hr) + bi
                    st['h'] = (hr, hi)
                    st['o'].append((hr, hi))
                    if len(st['o']) == 4:
                        (r0_, i0), (r1, i1), (r2, i2), (r3, i3) = st['o']
                        q = j // 4
                        cat = lambda a, b: jnp.concatenate([a, b], 0)
                        ur, ui, lr_, li_ = cat(r0_, r2), cat(i0, i2), cat(r1, r3), cat(i1, i3)
                        for n, v in enumerate(s_lhs32(ur, ui, lr_, li_)):
                            hs_s[n, 16 * q:16 * q + 16, ks] = v.astype(bf16)
                        st['o'] = []
                return f
            items.append(first)
            for j in range(L): items.append(p1(j))
            items.append(carry)
            for j in range(L): items.append(p2(j))
            return items

        cat0 = lambda l: jnp.concatenate(l, 0)
        cat1 = lambda l: jnp.concatenate(l, 1)

        def interleave(mx, va, lead=0.0):
            n = len(mx); done = 0
            for k, m in enumerate(mx):
                m()
                tgt = min(len(va), int(np.ceil((k + 1 + lead) * len(va) / n - 1e-9)))
                while done < tgt:
                    va[done](); done += 1
            while done < len(va):
                va[done](); done += 1

        @pl.when(step == 0)
        def _():
            cp = lambda src, dst, i: pltpu.make_async_copy(src, dst, sems.at[i])
            xcp = lambda i: cp(x_hbm.at[pl.ds(i * T1, T1)], x_s.at[pl.ds(i * T1, T1)], 16 + i)
            small = [cp(lre_hbm, lre_s, 0), cp(lim_hbm, lim_s, 1), cp(ldt_hbm, ldt_s, 2),
                     cp(dsk_hbm, dsk_s, 3), cp(gw_hbm, gw_s, 4)]
            c_bre = cp(bre_hbm, bre_s, 5); c_bim = cp(bim_hbm, bim_s, 6)
            c_cre = cp(cre_hbm, cre_s, 7); c_cim = cp(cim_hbm, cim_s, 8)
            c_wg = cp(wg_hbm, wg_s, 9); c_wu = cp(wu_hbm, wu_s, 10); c_wd = cp(wd_hbm, wd_s, 11)
            xcp(0).start(); c_bre.start(); c_bim.start()
            for c in small: c.start()
            for i in range(1, NX): xcp(i).start()
            c_wg.start(); c_wu.start(); c_cre.start(); c_cim.start(); c_wd.start()

            def comb_links(w1, w2, t_ref, nrows, zd):
                ch = {}
                its = []
                idx = 0
                for r in range(0, nrows, 16):
                    for c in range(2):
                        def f(r=r, c=c, key=0):
                            cs1 = slice(128 * c, 128 * c + 128); cs2 = slice(KH + 128 * c, KH + 128 * c + 128)
                            zb = zero_bits(ch[key], zd) if key in ch else None
                            g1 = gate16(w1[r:r + 16, cs1], zb); g2 = gate16(w1[r:r + 16, cs2], zb)
                            u1 = gate16(w2[r:r + 16, cs1], zb); u2 = gate16(w2[r:r + 16, cs2], zb)
                            v = s_rhs32(g1, u1, g2, u2)
                            for dst, src in enumerate((0, 2, 3, 5, 6)):
                                t_ref[dst, r:r + 16, cs1] = v[src].astype(bf16)
                            ch[key] = v[6][0:8]
                        its.append(f); idx += 1
                return its

            h1 = T1 // 2
            def prep_bu(i):
                r0 = i * T1
                its = []
                for q in range(0, h1, 16):
                    def f(q=q):
                        xu = x_s[pl.ds(r0 + q, 16), :].astype(f32)
                        xl = x_s[pl.ds(r0 + h1 + q, 16), :].astype(f32)
                        st4(xf_s, i, q, xu); st4(xf_s, i, h1 + q, xl)
                        for n, v in enumerate(s_lhs32(xu[:, :KH], xu[:, KH:], xl[:, :KH], xl[:, KH:])):
                            sb_s[i % 2, n, q:q + 16, :] = v.astype(bf16)
                    its.append(f)
                return its
            def bu_items(i):
                par = i % 2
                its = []
                for c in range(4):
                    def f(c=c):
                        cs = slice(128 * c, 128 * c + 128)
                        rhs = [tb_s[0, cs], bre_s[cs, :KH], tb_s[1, cs], tb_s[2, cs], bim_s[cs, KH:], tb_s[3, cs], tb_s[4, cs]]
                        m = [dnt(sb_s[par, n], rhs[n]) for n in range(7)]
                        c11, c12, c21, c22 = s_comb(m)
                        rr, ri = (b0r_s, b0i_s) if i * T1 < TM else (bur_s, bui_s)
                        for ref, rho, v in ((rr, 0, c11), (ri, 0, c12), (rr, h1, c21), (ri, h1, c22)):
                            for a_ in range(0, h1, 8):
                                ref[c, pl.ds(pos(i, rho + a_), 8), :] = v[a_:a_ + 8]
                    its.append(f)
                return its

            xcp(0).wait(); c_bre.wait()
            x0 = x_s[0:T1, :]
            st4(b0r_s, 0, 0, dnt(x0, bre_s[...]))
            st4(xf_s, 0, 0, x0.astype(f32))
            c_bim.wait()
            mx = [(lambda c=c: st4c(b0i_s, c, dnt(x0, bim_s[256 * c:256 * c + 256, :]))) for c in range(2)]
            def st4c(ref, c, v):
                for a in range(0, T1, 8):
                    off = pos(0, a)
                    for k in range(2):
                        ref[2 * c + k, pl.ds(off, 8), :] = v[a:a + 8, 128 * k:128 * k + 128]
            interleave(mx, comb_links(bre_s, bim_s, tb_s, P, zB))
            for c in small: c.wait()
            xcp(1).wait()
            for it in prep_bu(1): it()
            def params():
                lre = lre_s[...].astype(f32).reshape(1, P)
                lim = lim_s[...].astype(f32).reshape(1, P)
                dt = jnp.exp(ldt_s[...].astype(f32).reshape(1, P)).astype(bf16).astype(f32)
                are = dt * lre; aim = dt * lim
                row = lax.broadcasted_iota(jnp.int32, (8, P), 0)
                kk = jnp.where(row == 0, 1.0, jnp.where(row == 1, float(L), jnp.where(row == 2, float(2 * L), float(4 * L))))
                mag = jnp.exp(kk * are)
                pre = mag * jnp.cos(kk * aim); pim = mag * jnp.sin(kk * aim)
                bc = lambda v, i: jnp.broadcast_to(v[i:i + 1], (8, P))
                tab_s[0] = bc(pre, 0); tab_s[1] = bc(pim, 0)
                for n, d in enumerate((1, 2, 4)):
                    tab_s[2 + 2 * n] = jnp.where(row >= d, bc(pre, n + 1), 0.0)
                    tab_s[3 + 2 * n] = jnp.where(row >= d, bc(pim, n + 1), 0.0)
                tab_s[8] = jnp.where(row == 0, bc(pre, 1), 0.0)
                tab_s[9] = jnp.where(row == 0, bc(pim, 1), 0.0)
                nre = pre[0:1] - 1.0; nim = pim[0:1]
                den = lre * lre + lim * lim
                vec_s[2:3, :] = 2.0 * (nre * lre + nim * lim) / den
                vec_s[3:4, :] = 2.0 * (nim * lre - nre * lim) / den
                carry_s[...] = jnp.zeros((2, 8, P), f32)
                vec_s[0:1, :] = gw_s[...].astype(f32).reshape(1, D)
                vec_s[1:2, :] = dsk_s[...].astype(f32).reshape(1, D)
            xcp(2).wait()
            interleave(bu_items(1), [params] + prep_bu(2))
            for i in range(3, NX): xcp(i).wait()
            l0 = [scan_lane(0, k, None, b0r_s, b0i_s) for k in range(4)]
            sA = merge2(l0[0], l0[1]); sB = merge2(l0[2], l0[3])
            interleave(bu_items(2), merge2(prep_bu(3), sA))
            interleave(bu_items(3), merge2(prep_bu(4), sB))
            interleave(bu_items(4), prep_bu(5))
            c_wg.wait(); c_wu.wait()
            gu = comb_links(wg_s, wu_s, tf_s, F, zG)
            n6, n7 = int(n6f * len(gu)), int(n7f * len(gu))
            interleave(bu_items(5), merge2(prep_bu(6), gu[:n6]))
            interleave(bu_items(6), merge2(prep_bu(7), gu[n6:n7]))
            c_cre.wait(); c_cim.wait(); c_wd.wait()
            chc = {}
            def cpr(r, c, key):
                def f():
                    cs = slice(128 * c, 128 * c + 128)
                    fre = vec_s[2:3, cs]; fim = vec_s[3:4, cs]
                    zb = zero_bits(chc[key], zC) if key in chc else None
                    a1 = gate16(cre_s[r:r + 16, cs], zb); b1 = gate16(cim_s[r:r + 16, cs], zb)
                    a2 = gate16(cre_s[256 + r:272 + r, cs], zb); b2 = gate16(cim_s[256 + r:272 + r, cs], zb)
                    r1 = a1 * fre - b1 * fim; i1 = -(a1 * fim + b1 * fre)
                    r2 = a2 * fre - b2 * fim; i2 = -(a2 * fim + b2 * fre)
                    v = s_rhs32(r1, r2, i1, i2)
                    for n in range(7):
                        tc_s[n, r:r + 16, cs] = v[n].astype(bf16)
                    chc[key] = v[0][0:8]
                return f
            cps = [cpr(r, c, 0) for r in range(0, 256, 16) for c in range(4)]
            interleave(bu_items(7), merge2(cps, gu[n7:]))
        pb = step * (8 * LP)
        xu = cat0([ld(xf_s, pb, 2 * m) for m in range(L // 2)])
        xl = cat0([ld(xf_s, pb, 2 * m + 1) for m in range(L // 2)])
        sa = [v.astype(bf16) for v in s_lhs32(xu[:, :KH], xu[:, KH:], xl[:, :KH], xl[:, KH:])]

        def stage2a():
            m = [dnt(hs_s[n], tc_s[n]) for n in range(7)]
            c11, c12, c21, c22 = s_comb(m)
            return cat0([cat1([c11, c12]), cat1([c21, c22])])

        def ffn_cols(c0, c1):
            m = [dnt(sa[0], tf_s[0, c0:c1]), dnt(sa[1], wg_s[c0:c1, :KH]), dnt(sa[2], tf_s[1, c0:c1]),
                 dnt(sa[3], tf_s[2, c0:c1]), dnt(sa[4], wu_s[c0:c1, KH:]), dnt(sa[5], tf_s[3, c0:c1]),
                 dnt(sa[6], tf_s[4, c0:c1])]
            c11, c12, c21, c22 = s_comb(m)
            return _gelu(c11) * c12, _gelu(c21) * c22

        ya = stage2a()
        nxt = jnp.minimum(step + 1, NB - 1)
        chunks = [(c, min(c + CW, F)) for c in range(0, F, CW)]
        acts = []
        for ci_, (c0, c1) in enumerate(chunks):
            au, al = ffn_cols(c0, c1)
            for k in [k for k in range(4) if stagger[k] == ci_]:
                for it in scan_lane(nxt, k, lambda v=au: v[0:8, 0:128]):
                    it()
            acts.append(cat0([au, al]).astype(bf16))
        act = cat1(acts)
        xp = cat0([xu, xl])
        g = jax.nn.sigmoid(jnp.sum(xp * vec_s[0:1, :], axis=-1, keepdims=True))
        u = g * (ya + xp * vec_s[1:2, :])
        w = 1.0 - g
        for k in range(4 // dw):
            cs = slice(128 * dw * k, 128 * dw * (k + 1))
            ybk = dnn(act, wd_s[:, cs])
            res = u[:, cs] + w * ybk
            for kk in range(dw):
                kc = dw * k + kk
                for pr in range(2):
                    for m_ in range(L // 2):
                        r = pr * H + 8 * m_
                        ot_s[kc, pl.ds(2 * m_ + pr, 8, stride=LP), :] = res[r:r + 8, 128 * kk:128 * kk + 128]
                for c in range(8):
                    o_ref[c * L:(c + 1) * L, 128 * kc:128 * kc + 128] = ot_s[kc, c * LP:c * LP + L, :].astype(odt)

    @jax.jit
    def fn(A_x, A_Lambda_re, A_Lambda_im, A_B_re, A_B_im, A_C_re, A_C_im, A_log_dt, A_Dskip,
           B_x, B_w_gate, B_w_up, B_w_down, gate_w):
        anyspec = pl.BlockSpec(memory_space=pl.ANY)
        V = pltpu.VMEM
        out = pl.pallas_call(
            kern,
            grid=(NB,),
            in_specs=[anyspec] * 13,
            out_specs=pl.BlockSpec((TM, D), lambda i: (i, 0)),
            out_shape=jax.ShapeDtypeStruct((S, D), odt),
            scratch_shapes=[V((S, D), bf16), V((P,), bf16), V((P,), bf16), V((P,), bf16), V((D,), bf16), V((D,), bf16),
                            V((P, D), bf16), V((P, D), bf16), V((D, P), bf16), V((D, P), bf16),
                            V((F, D), bf16), V((F, D), bf16), V((F, D), bf16),
                            V((4, SP, 128), f32), V((4, SP, 128), f32), V((4, SP, 128), f32), V((4, 8 * LP, 128), f32),
                            V((10, 8, P), f32), V((2, 8, P), f32), V((8, D), f32),
                            V((5, F, KH), bf16), V((5, P, KH), bf16), V((7, 256, P), bf16),
                            V((7, H, P), bf16), V((2, 7, T1 // 2, KH), bf16),
                            V((4, 8 * LP, 128), f32), V((4, 8 * LP, 128), f32),
                            pltpu.SemaphoreType.DMA((16 + NX,))],
            compiler_params=pltpu.CompilerParams(dimension_semantics=("arbitrary",),
                                                 vmem_limit_bytes=100 * 1024 * 1024),
        )(A_x.reshape(S, D), A_Lambda_re, A_Lambda_im, A_B_re, A_B_im, A_C_re, A_C_im,
          A_log_dt, A_Dskip, B_w_gate.T, B_w_up.T, B_w_down, gate_w)
        return out.reshape(1, S, D)
    return fn


_kernel_fn = _build()


@jax.jit
def pallas_gated_mix__ssm_conv_s5__geglu_ffn__prompt_kernel(
    A_x, A_Lambda_re, A_Lambda_im, A_B_re, A_B_im, A_C_re, A_C_im, A_log_dt, A_Dskip,
    B_x, B_w_gate, B_w_up, B_w_down, gate_w,
):
    return _kernel_fn(A_x, A_Lambda_re, A_Lambda_im, A_B_re, A_B_im, A_C_re, A_C_im, A_log_dt, A_Dskip,
                      B_x, B_w_gate, B_w_up, B_w_down, gate_w)
```
